```python
import os as _os
_os.environ.setdefault('JAX_PLATFORMS', 'cpu')
import jax
import jax.numpy as jnp

def _softmax(x, axis=-1):
    return jax.nn.softmax(x, axis=axis)

def _gelu(x):
    return jax.nn.gelu(x, approximate=True)

def _silu(x):
    return jax.nn.silu(x)

def _sigmoid(x):
    return jax.nn.sigmoid(x)

def _layernorm(x, axis=-1, eps=1e-05):
    m = jnp.mean(x, axis=axis, keepdims=True)
    v = jnp.var(x, axis=axis, keepdims=True)
    return (x - m) / jnp.sqrt(v + eps)

def _scatter_add(tgt, idx, src, axis=0):
    return tgt.at[idx].add(src)

def _segment_sum(src, seg, n):
    return jax.ops.segment_sum(src, seg, n)

class _Rng:

    def __init__(self, key):
        self._k = key

    def _next(self):
        self._k, sub = jax.random.split(self._k)
        return sub

    def normal(self, shape):
        return jax.random.normal(self._next(), shape, dtype=jnp.bfloat16)

    def randint(self, lo, hi, shape):
        return jax.random.randint(self._next(), shape, lo, hi, dtype=jnp.int32)

    def uniform(self, shape, lo=0.0, hi=1.0):
        return jax.random.uniform(self._next(), shape, jnp.bfloat16, lo, hi)

    def permutation(self, n):
        return jax.random.permutation(self._next(), n)
kernel_name = 'parallel_sum__memory_aug_recurrent_mem_tr__dense_activation_gelu__prompt'

def setup_inputs():
    _rng = _Rng(jax.random.key(int.from_bytes(__import__("os").urandom(4), "little")))
    _w = lambda a: (lambda t: t.astype(jnp.bfloat16) if jnp.issubdtype(t.dtype, jnp.floating) else t)(jnp.asarray(a))

    def _A_setup():
        B, S, Dm = (1, 2048, 1024)
        H, Dh = (32, 128)
        M, seg = (8, 32)
        seg = min(seg, S)
        S = S // seg * seg
        return {'x': _w((lambda *s: _rng.normal(s) * 0.05)(B, S, Dm)), 'mem0': _w((lambda *s: _rng.normal(s) * 0.2)(B, M, Dm)), 'Wq': _w((lambda *s: _rng.normal(s) * 0.8)(Dm, H, Dh) * Dm ** (-0.5)), 'Wk': _w((lambda *s: _rng.normal(s) * 0.8)(Dm, H, Dh) * Dm ** (-0.5)), 'Wv': _w((lambda *s: _rng.normal(s) * 0.2)(Dm, H, Dh) * Dm ** (-0.5)), 'Wo': _w((lambda *s: _rng.normal(s) * 0.2)(H, Dh, Dm) * (H * Dh) ** (-0.5)), 'seg_len': seg}
    _A_in = _A_setup()

    def _B_setup():
        B, S, D, F = (1, 2048, 1024, 3584)
        return {'x': _w((lambda *s: _rng.normal(s) * 0.05)(B, S, D)), 'w1': _w((lambda *s: _rng.normal(s) * 0.1)(D, F) * D ** (-0.5)), 'b1': _w((lambda *s: _rng.normal(s) * 0.1)(F) * 0.01), 'w2': _w((lambda *s: _rng.normal(s) * 0.1)(F, D) * F ** (-0.5)), 'b2': _w((lambda *s: _rng.normal(s) * 0.05)(D) * 0.01)}
    _B_in = _B_setup()
    return {'A_x': _A_in['x'], 'A_mem0': _A_in['mem0'], 'A_Wq': _A_in['Wq'], 'A_Wk': _A_in['Wk'], 'A_Wv': _A_in['Wv'], 'A_Wo': _A_in['Wo'], 'A_seg_len': _A_in['seg_len'], 'B_x': _B_in['x'], 'B_w1': _B_in['w1'], 'B_b1': _B_in['b1'], 'B_w2': _B_in['w2'], 'B_b2': _B_in['b2']}

def reference(A_x, A_mem0, A_Wq, A_Wk, A_Wv, A_Wo, A_seg_len, B_x, B_w1, B_b1, B_w2, B_b2):

    def _A_ref(x, mem0, Wq, Wk, Wv, Wo, seg_len):
        B, S, Dm = x.shape
        H, Dh = (Wq.shape[1], Wq.shape[2])
        M = mem0.shape[1]
        scale = Dh ** (-0.5)
        n_seg = S // seg_len
        L = M + seg_len
        idx = jnp.arange(L)
        mask = (idx[:, None] < M) | (idx[:, None] >= idx[None, :])
        mem = mem0
        outs = []
        for s in range(n_seg):
            xs = x[:, s * seg_len:(s + 1) * seg_len, :].copy()
            h = jnp.concatenate([mem, xs], axis=1)
            q = jnp.einsum('btd,dhe->bhte', h, Wq)
            k = jnp.einsum('btd,dhe->bhte', h, Wk)
            v = jnp.einsum('btd,dhe->bhte', h, Wv)
            scores = jnp.einsum('bhqe,bhke->bhqk', q, k) * scale
            scores = jnp.where(mask[None, None], scores, -1000000000.0)
            p = _softmax(scores, axis=-1)
            o = jnp.einsum('bhqk,bhke->bhqe', p, v)
            o = jnp.einsum('bhte,hed->btd', o, Wo)
            mem = o[:, :M, :].copy()
            outs.append(o[:, M:, :])
        return jnp.concatenate(outs, axis=1)

    def _B_ref(x, w1, b1, w2, b2):
        h = jnp.einsum('bsd,df->bsf', x, w1) + b1
        h = _gelu(h)
        return jnp.einsum('bsf,fd->bsd', h, w2) + b2
    x = A_x
    xn = _layernorm(x, axis=-1)
    return x + _A_ref(xn, A_mem0, A_Wq, A_Wk, A_Wv, A_Wo, A_seg_len) + _B_ref(xn, B_w1, B_b1, B_w2, B_b2)
```

```python
import functools

import jax
import jax.numpy as jnp
import numpy as np
from jax import lax
from jax.experimental import pallas as pl
from jax.experimental.pallas import tpu as pltpu

_F32 = jnp.float32
_BF16 = jnp.bfloat16


def _dot(a, b):
    return jnp.dot(a, b, preferred_element_type=_F32)


def _dot_nt(a, b):
    return lax.dot_general(a, b, (((1,), (1,)), ((), ())), preferred_element_type=_F32)


def _make_kernel(S, D, H, E, M, SEG, F, FC, scale):
    NSEG = S // SEG
    L = M + SEG
    LP = 48
    RIDE = 32 - M
    REST = SEG - RIDE
    NFC = F // FC
    NDC = D // 128
    NT = D // 128
    PH = 2
    NP = H // PH
    WLAG = 3
    SB = 8
    NRB = NSEG // SB
    RB = SB * SEG

    def kernel(x_ref, mem0_ref, b1_ref, b2_ref,
               wq_hbm, wk_hbm, wv_hbm, wo_hbm, w1_hbm, w2_hbm,
               out_ref,
               wqkv_v, wo_v, xn_v, xpre_v, acc_v,
               sem_w1, sem_w2, sem_wo, sem_st):
        w_hbm = (wq_hbm, wk_hbm, wv_hbm)

        def phase1(w1_v, w2_v, stage_v):
            def w1_copy(j):
                return pltpu.make_async_copy(
                    w1_hbm.at[:, pl.ds(j * FC, FC)], w1_v.at[j], sem_w1.at[j])

            def w2_copy(j):
                return pltpu.make_async_copy(
                    w2_hbm.at[pl.ds(j * FC, FC), :], w2_v.at[j], sem_w2.at[j])

            def st_copy(c, slot, p):
                return pltpu.make_async_copy(
                    w_hbm[p].at[pl.ds(c * 128, 128)], stage_v.at[slot, p],
                    sem_st.at[slot, p])

            def wo_copy(j):
                return pltpu.make_async_copy(
                    wo_hbm.at[:, pl.ds(j * 128, 128)], wo_v.at[j], sem_wo.at[j])

            w1_copy(0).start()
            w2_copy(0).start()
            for p in range(3):
                st_copy(0, 0, p).start()
            w1_copy(1).start()
            w2_copy(1).start()
            for p in range(3):
                st_copy(1, 1, p).start()
            for j in range(2, NFC):
                w1_copy(j).start()
                w2_copy(j).start()
            for j in range(NT):
                wo_copy(j).start()

            b2 = b2_ref[...].astype(_F32)

            def ln_body(i, carry):
                r = pl.ds(pl.multiple_of(i * SB, SB), SB)
                xb = x_ref[r].astype(_F32)
                mu = jnp.mean(xb, axis=-1, keepdims=True)
                xc = xb - mu
                var = jnp.mean(xc * xc, axis=-1, keepdims=True)
                xn = xc * lax.rsqrt(var + 1e-5)
                xn_v[r] = xn.astype(_BF16)
                xpre_v[r] = xn[:, RIDE:, :]
                acc_v[r] = xb + b2
                return carry

            lax.fori_loop(0, NRB, ln_body, 0)

            def relayout(c, slot, p):
                blk = stage_v[slot, p]
                wqkv_v[pl.ds(p * H, H), pl.ds(pl.multiple_of(c * 128, 128), 128), :] = (
                    jnp.swapaxes(blk, 0, 1))

            def fc_body(j, carry):
                slot = j % 2
                w1_copy(j).wait()
                w2_copy(j).wait()
                for p in range(3):
                    st_copy(j, slot, p).wait()
                b1 = b1_ref[j].astype(_F32)
                for rb in range(NRB):
                    xb = xn_v[pl.ds(rb * SB, SB)].reshape(RB, D)
                    h = _dot(xb, w1_v[j]) + b1
                    h = jax.nn.gelu(h, approximate=True).astype(_BF16)
                    y = _dot(h, w2_v[j])
                    acc_v[pl.ds(rb * SB, SB)] += y.reshape(SB, SEG, D)
                    if rb in (1, 3, 5):
                        relayout(j, slot, (rb - 1) // 2)

                @pl.when(j + 2 < NDC)
                def _():
                    for p in range(3):
                        st_copy(j + 2, slot, p).start()

                return carry

            lax.fori_loop(0, NFC, fc_body, 0)
            for c in range(NFC, NDC):
                for p in range(3):
                    st_copy(c, c % 2, p).wait()
                    relayout(c, c % 2, p)
            for j in range(NT):
                wo_copy(j).wait()

        pl.run_scoped(
            phase1,
            pltpu.VMEM((NFC, D, FC), _BF16),
            pltpu.VMEM((NFC, FC, D), _BF16),
            pltpu.VMEM((2, 3, 128, H, E), _BF16),
        )

        def phase2(qkvpre_v, opost_v, xl_v, wacc_v):
            xl_v[...] = xpre_v[...].reshape(NSEG * REST, D).astype(_BF16)

            def pre_body(sg, carry):
                for t in range(8):
                    slab = sg * 8 + t
                    y = _dot(xl_v[...], wqkv_v[slab])
                    qkvpre_v[slab] = y.reshape(NSEG, REST, E)
                return carry

            lax.fori_loop(0, 3 * H // 8, pre_body, 0)

            row = lax.broadcasted_iota(jnp.int32, (LP, LP), 0)
            col = lax.broadcasted_iota(jnp.int32, (LP, LP), 1)
            mask = ((row < M) | (row >= col)) & (col < L)
            zpad = jnp.zeros((LP - L, E), _F32)

            def seg_body(s, mem):
                xs = xn_v[s].astype(_F32)
                lhs = jnp.concatenate([mem, xs[:RIDE]], axis=0).astype(_BF16)

                qkv = [{}, {}, {}]
                sc, mx, ex, den, ob = {}, {}, {}, {}, {}

                def heads(i):
                    return range(i * PH, (i + 1) * PH)

                def stage_a(p, i):
                    for h in heads(i):
                        y = _dot(lhs, wqkv_v[p * H + h])
                        qkv[p][h] = jnp.concatenate(
                            [y, qkvpre_v[p * H + h, s], zpad], axis=0).astype(_BF16)

                def stage_1(i):
                    for h in heads(i):
                        sc[h] = _dot_nt(qkv[0].pop(h), qkv[1].pop(h))

                def stage_2(i):
                    for h in heads(i):
                        sc[h] = jnp.where(mask, sc[h] * scale, -1000000000.0)
                        mx[h] = jnp.max(sc[h], axis=-1, keepdims=True)

                def stage_3(i):
                    for h in heads(i):
                        ex[h] = jnp.exp(sc.pop(h) - mx.pop(h))
                        den[h] = jnp.sum(ex[h], axis=-1, keepdims=True)

                def stage_4(i):
                    for h in heads(i):
                        p_ = (ex.pop(h) / den.pop(h)).astype(_BF16)
                        o = _dot(p_, qkv[2].pop(h))
                        ob[h] = o[:32].astype(_BF16)
                        opost_v[s, :, pl.ds(h * E, E)] = o[32:L]

                def stage_w(i):
                    og = jnp.concatenate([ob.pop(h) for h in heads(i)], axis=1)
                    for j in range(NT):
                        y = _dot(og, wo_v[j, pl.ds(i * PH * E, PH * E), :])
                        if i == 0:
                            wacc_v[:, pl.ds(j * 128, 128)] = y
                        else:
                            wacc_v[:, pl.ds(j * 128, 128)] += y

                for p in range(3):
                    stage_a(p, 0)
                for i in range(NP):
                    last = i == NP - 1
                    stage_1(i)
                    if last:
                        stage_w(i - 3)
                    else:
                        stage_a(0, i + 1)
                    stage_2(i)
                    if last:
                        stage_w(i - 2)
                    else:
                        stage_a(1, i + 1)
                    stage_3(i)
                    if last:
                        stage_w(i - 1)
                    else:
                        stage_a(2, i + 1)
                        if i >= WLAG:
                            stage_w(i - WLAG)
                    stage_4(i)
                stage_w(NP - 1)

                out32 = wacc_v[...]
                acc_v[s, pl.ds(0, RIDE), :] += out32[M:]
                return out32[:M]

            lax.fori_loop(0, NSEG, seg_body, mem0_ref[...].astype(_F32))

            PB = 16
            for rb in range(NSEG // PB):
                ol = opost_v[pl.ds(rb * PB, PB)].reshape(PB * REST, H * E).astype(_BF16)
                for j in range(NT):
                    y = _dot(ol, wo_v[j])
                    acc_v[pl.ds(rb * PB, PB), pl.ds(RIDE, REST), pl.ds(j * 128, 128)] += (
                        y.reshape(PB, REST, 128))

            def out_body(i, carry):
                r = pl.ds(pl.multiple_of(i * SB, SB), SB)
                out_ref[r] = acc_v[r].astype(out_ref.dtype)
                return carry

            lax.fori_loop(0, NRB, out_body, 0)

        pl.run_scoped(
            phase2,
            pltpu.VMEM((3 * H, NSEG, REST, E), _F32),
            pltpu.VMEM((NSEG, REST, H * E), _F32),
            pltpu.VMEM((NSEG * REST, D), _BF16),
            pltpu.VMEM((32, D), _F32),
        )

    scratch = [
        pltpu.VMEM((3 * H, D, E), _BF16),
        pltpu.VMEM((NT, H * E, 128), _BF16),
        pltpu.VMEM((NSEG, SEG, D), _BF16),
        pltpu.VMEM((NSEG, REST, D), _F32),
        pltpu.VMEM((NSEG, SEG, D), _F32),
        pltpu.SemaphoreType.DMA((NFC,)),
        pltpu.SemaphoreType.DMA((NFC,)),
        pltpu.SemaphoreType.DMA((NT,)),
        pltpu.SemaphoreType.DMA((2, 3)),
    ]
    return kernel, scratch


@functools.partial(jax.jit, static_argnames=("A_seg_len",))
def pallas_parallel_sum__memory_aug_recurrent_mem_tr__dense_activation_gelu__prompt_kernel(
    A_x: jax.Array,
    A_mem0: jax.Array,
    A_Wq: jax.Array,
    A_Wk: jax.Array,
    A_Wv: jax.Array,
    A_Wo: jax.Array,
    A_seg_len: int,
    B_x: jax.Array,
    B_w1: jax.Array,
    B_b1: jax.Array,
    B_w2: jax.Array,
    B_b2: jax.Array,
):
    del B_x
    B, S, D = A_x.shape
    H, E = A_Wq.shape[1], A_Wq.shape[2]
    M = A_mem0.shape[1]
    SEG = int(A_seg_len)
    F = B_w1.shape[1]
    FC = 512
    assert B == 1 and M == 8 and SEG == 32 and E == 128
    assert S % (8 * SEG) == 0 and D % 128 == 0 and H % 8 == 0
    assert F % FC == 0 and F // FC == D // 128 - 1
    NSEG = S // SEG

    scale = float(np.asarray(E ** (-0.5)).astype(A_x.dtype).astype(np.float32))

    kernel, scratch = _make_kernel(S, D, H, E, M, SEG, F, FC, scale)

    vmem = pl.BlockSpec(memory_space=pltpu.VMEM)
    hbm = pl.BlockSpec(memory_space=pl.ANY)
    out = pl.pallas_call(
        kernel,
        out_shape=jax.ShapeDtypeStruct((NSEG, SEG, D), A_x.dtype),
        in_specs=[vmem, vmem, vmem, vmem, hbm, hbm, hbm, hbm, hbm, hbm],
        out_specs=vmem,
        scratch_shapes=scratch,
        compiler_params=pltpu.CompilerParams(vmem_limit_bytes=120 * 1024 * 1024),
    )(
        A_x.reshape(NSEG, SEG, D),
        A_mem0.reshape(M, D),
        B_b1.reshape(F // FC, 1, FC),
        B_b2.reshape(1, D),
        A_Wq, A_Wk, A_Wv,
        A_Wo.reshape(H * E, D),
        B_w1, B_w2,
    )
    return out.reshape(B, S, D)
```

```python
import functools

import jax
import jax.numpy as jnp
import numpy as np
from jax import lax
from jax.experimental import pallas as pl
from jax.experimental.pallas import tpu as pltpu

_F32 = jnp.float32
_BF16 = jnp.bfloat16


def _dot(a, b):
    return jnp.dot(a, b, preferred_element_type=_F32)


def _dot_nt(a, b):
    return lax.dot_general(a, b, (((1,), (1,)), ((), ())), preferred_element_type=_F32)


def _make_kernel(S, D, H, E, M, SEG, F, FC, FT, scale):
    NSEG = S // SEG
    L = M + SEG
    LP = 48
    RIDE = 32 - M
    REST = SEG - RIDE
    NFC = (F - FT) // FC
    NTF = FT // 128
    F0 = NFC * FC
    NDC = D // 128
    NT = D // 128
    PH = 2
    NP = H // PH
    WLAG = 3
    SB = 8
    NRB = NSEG // SB
    RB = SB * SEG
    PB = 16
    NPB = NSEG // PB

    def kernel(x_hbm, mem0_ref, b1_ref, b2_ref,
               wq_hbm, wk_hbm, wv_hbm, wo_hbm, w1_hbm, w2_hbm,
               out_hbm,
               wqkv_v, wo_v, w1t_v, w2t_v, xn_v, xpre_v, acc_v,
               sem_x, sem_w1, sem_w2, sem_wo, sem_st, sem_w1t, sem_w2t, sem_out):
        w_hbm = (wq_hbm, wk_hbm, wv_hbm)

        def phase1(x_v, w1_v, w2_v, stage_v):
            def x_copy(i):
                r = pl.ds(i * SB, SB)
                return pltpu.make_async_copy(x_hbm.at[r], x_v.at[r], sem_x.at[i])

            def w1_copy(j):
                return pltpu.make_async_copy(
                    w1_hbm.at[:, pl.ds(j * FC, FC)], w1_v.at[j], sem_w1.at[j])

            def w2_copy(j):
                return pltpu.make_async_copy(
                    w2_hbm.at[pl.ds(j * FC, FC), :], w2_v.at[j], sem_w2.at[j])

            def st_copy(c, slot, p):
                return pltpu.make_async_copy(
                    w_hbm[p].at[pl.ds(c * 128, 128)], stage_v.at[slot, p],
                    sem_st.at[slot, p])

            def wo_copy(j):
                return pltpu.make_async_copy(
                    wo_hbm.at[:, pl.ds(j * 128, 128)], wo_v.at[j], sem_wo.at[j])

            def w1t_copy(t):
                return pltpu.make_async_copy(
                    w1_hbm.at[:, pl.ds(F0 + t * 128, 128)], w1t_v.at[t], sem_w1t.at[t])

            def w2t_copy(j):
                return pltpu.make_async_copy(
                    w2_hbm.at[pl.ds(F0, FT), pl.ds(j * 128, 128)], w2t_v.at[j],
                    sem_w2t.at[j])

            for i in range(NRB):
                x_copy(i).start()
            w1_copy(0).start()
            w2_copy(0).start()

            b2 = b2_ref[...].astype(_F32)

            def ln_body(i, carry):
                x_copy(i).wait()
                r = pl.ds(pl.multiple_of(i * SB, SB), SB)
                xb = x_v[r].astype(_F32)
                mu = jnp.mean(xb, axis=-1, keepdims=True)
                xc = xb - mu
                var = jnp.mean(xc * xc, axis=-1, keepdims=True)
                xn = xc * lax.rsqrt(var + 1e-5)
                xn_v[r] = xn.astype(_BF16)
                xpre_v[r] = xn[:, RIDE:, :]
                acc_v[r] = xb + b2
                return carry

            lax.fori_loop(0, NRB // 2, ln_body, 0)
            for p in range(3):
                st_copy(0, 0, p).start()
            w1_copy(1).start()
            w2_copy(1).start()
            for p in range(3):
                st_copy(1, 1, p).start()
            lax.fori_loop(NRB // 2, NRB, ln_body, 0)
            for j in range(2, NFC):
                w1_copy(j).start()
                w2_copy(j).start()
            for j in range(NT):
                wo_copy(j).start()
            for t in range(NTF):
                w1t_copy(t).start()
            for j in range(NT):
                w2t_copy(j).start()

            def relayout(c, slot, p, q):
                blk = stage_v[slot, p, pl.ds(q * 16, 16)]
                d0 = pl.multiple_of(c * 128 + q * 16, 16)
                wqkv_v[pl.ds(p * H, H), pl.ds(d0, 16), :] = jnp.swapaxes(blk, 0, 1)

            def fc_body(j, carry):
                slot = j % 2
                w1_copy(j).wait()
                w2_copy(j).wait()
                b1 = b1_ref[:, pl.ds(pl.multiple_of(j * FC, 128), FC)].astype(_F32)
                for rb in range(NRB):
                    if rb == 2:
                        for p in range(3):
                            st_copy(j, slot, p).wait()
                    xb = xn_v[pl.ds(rb * SB, SB)].reshape(RB, D)
                    u0 = 4 * (rb - 2)
                    if rb >= 2:
                        for u in range(u0, u0 + 2):
                            relayout(j, slot, u % 3, u // 3)
                    h = _dot(xb, w1_v[j]) + b1
                    h = jax.nn.gelu(h, approximate=True).astype(_BF16)
                    if rb >= 2:
                        for u in range(u0 + 2, u0 + 4):
                            relayout(j, slot, u % 3, u // 3)
                    y = _dot(h, w2_v[j])
                    acc_v[pl.ds(rb * SB, SB)] += y.reshape(SB, SEG, D)

                @pl.when(j + 2 < NDC)
                def _():
                    for p in range(3):
                        st_copy(j + 2, slot, p).start()

                return carry

            lax.fori_loop(0, NFC, fc_body, 0)
            for j in range(NT):
                wo_copy(j).wait()
                w2t_copy(j).wait()
            for t in range(NTF):
                w1t_copy(t).wait()

        pl.run_scoped(
            phase1,
            pltpu.VMEM((NSEG, SEG, D), _BF16),
            pltpu.VMEM((NFC, D, FC), _BF16),
            pltpu.VMEM((NFC, FC, D), _BF16),
            pltpu.VMEM((2, 3, 128, H, E), _BF16),
        )

        def phase2(qkvpre_v, opost_v, xl_v, wacc_v, obuf_v):
            xl_v[...] = xpre_v[...].reshape(NSEG * REST, D).astype(_BF16)

            def pre_body(sg, carry):
                for t in range(8):
                    slab = sg * 8 + t
                    y = _dot(xl_v[...], wqkv_v[slab])
                    qkvpre_v[slab] = y.reshape(NSEG, REST, E)
                return carry

            lax.fori_loop(0, 3 * H // 8, pre_body, 0)

            row = lax.broadcasted_iota(jnp.int32, (LP, LP), 0)
            col = lax.broadcasted_iota(jnp.int32, (LP, LP), 1)
            mask = ((row < M) | (row >= col)) & (col < L)
            zpad = jnp.zeros((LP - L, E), _F32)
            b1t = b1_ref[:, pl.ds(F0, FT)].astype(_F32)

            def seg_body(s, mem):
                xsb = xn_v[s]
                lhs = jnp.concatenate(
                    [mem, xsb.astype(_F32)[:RIDE]], axis=0).astype(_BF16)

                qkv = [{}, {}, {}]
                sc, mx, ex, den, pr, ob = {}, {}, {}, {}, {}, {}

                def heads(i):
                    return range(i * PH, (i + 1) * PH)

                def stage_a(p, i):
                    for h in heads(i):
                        y = _dot(lhs, wqkv_v[p * H + h])
                        qkv[p][h] = jnp.concatenate(
                            [y, qkvpre_v[p * H + h, s], zpad], axis=0).astype(_BF16)

                def stage_1(i):
                    for h in heads(i):
                        sc[h] = _dot_nt(qkv[0].pop(h), qkv[1].pop(h))

                def stage_2(i):
                    for h in heads(i):
                        sc[h] = jnp.where(mask, sc[h] * scale, -1000000000.0)
                        mx[h] = jnp.max(sc[h], axis=-1, keepdims=True)

                def stage_3(i):
                    for h in heads(i):
                        ex[h] = jnp.exp(sc.pop(h) - mx.pop(h))
                        den[h] = jnp.sum(ex[h], axis=-1, keepdims=True)

                def stage_4(i):
                    for h in heads(i):
                        d = den.pop(h)
                        r = pl.reciprocal(d, approx=True)
                        r = r * (2.0 - d * r)
                        pr[h] = (ex.pop(h) * r).astype(_BF16)

                def stage_5(i):
                    for h in heads(i):
                        o = _dot(pr.pop(h), qkv[2].pop(h))
                        ob[h] = o[:32].astype(_BF16)
                        opost_v[s, :, pl.ds(h * E, E)] = o[32:L]

                def stage_w(i):
                    og = jnp.concatenate([ob.pop(h) for h in heads(i)], axis=1)
                    for j in range(NT):
                        y = _dot(og, wo_v[j, pl.ds(i * PH * E, PH * E), :])
                        if i == 0:
                            wacc_v[:, pl.ds(j * 128, 128)] = y
                        else:
                            wacc_v[:, pl.ds(j * 128, 128)] += y

                hm, ym, gl = {}, {}, []

                def stage_m1(t):
                    hm[t] = _dot(xsb, w1t_v[t])

                def stage_mg():
                    hh = jnp.concatenate([hm.pop(t) for t in range(NTF)], axis=1) + b1t
                    gl.append(jax.nn.gelu(hh, approximate=True).astype(_BF16))

                def stage_m2(j):
                    ym[j] = _dot(gl[0], w2t_v[j])

                for p in range(3):
                    stage_a(p, 0)
                for i in range(NP):
                    last = i == NP - 1
                    stage_1(i)
                    if last:
                        stage_w(i - 3)
                    else:
                        stage_a(0, i + 1)
                    stage_2(i)
                    if last:
                        stage_w(i - 2)
                    else:
                        stage_a(1, i + 1)
                    stage_3(i)
                    if last:
                        stage_w(i - 1)
                    else:
                        stage_a(2, i + 1)
                    stage_4(i)
                    if last:
                        for j in range(2, 5):
                            stage_m2(j)
                    elif i >= WLAG:
                        stage_w(i - WLAG)
                    elif i < 2:
                        stage_m1(2 * i)
                        stage_m1(2 * i + 1)
                    else:
                        stage_mg()
                        stage_m2(0)
                        stage_m2(1)
                    stage_5(i)
                for j in range(5, NT):
                    stage_m2(j)
                stage_w(NP - 1)

                out32 = wacc_v[...]
                ymlp = jnp.concatenate([ym.pop(j) for j in range(NT)], axis=1)
                acc_v[s, pl.ds(0, RIDE), :] += out32[M:] + ymlp[:RIDE]
                acc_v[s, pl.ds(RIDE, REST), :] += ymlp[RIDE:]
                return out32[:M]

            lax.fori_loop(0, NSEG, seg_body, mem0_ref[...].astype(_F32))

            def out_copy(rb):
                return pltpu.make_async_copy(
                    obuf_v.at[rb % 2], out_hbm.at[pl.ds(rb * PB, PB)], sem_out.at[rb % 2])

            for rb in range(NPB):
                ol = opost_v[pl.ds(rb * PB, PB)].reshape(PB * REST, H * E).astype(_BF16)
                for j in range(NT):
                    y = _dot(ol, wo_v[j])
                    acc_v[pl.ds(rb * PB, PB), pl.ds(RIDE, REST), pl.ds(j * 128, 128)] += (
                        y.reshape(PB, REST, 128))
                if rb >= 2:
                    out_copy(rb - 2).wait()
                obuf_v[rb % 2] = acc_v[pl.ds(rb * PB, PB)].astype(obuf_v.dtype)
                out_copy(rb).start()
            for rb in range(NPB - 2, NPB):
                out_copy(rb).wait()

        pl.run_scoped(
            phase2,
            pltpu.VMEM((3 * H, NSEG, REST, E), _F32),
            pltpu.VMEM((NSEG, REST, H * E), _F32),
            pltpu.VMEM((NSEG * REST, D), _BF16),
            pltpu.VMEM((32, D), _F32),
            pltpu.VMEM((2, PB, SEG, D), _BF16),
        )

    scratch = [
        pltpu.VMEM((3 * H, D, E), _BF16),
        pltpu.VMEM((NT, H * E, 128), _BF16),
        pltpu.VMEM((NTF, D, 128), _BF16),
        pltpu.VMEM((NT, FT, 128), _BF16),
        pltpu.VMEM((NSEG, SEG, D), _BF16),
        pltpu.VMEM((NSEG, REST, D), _F32),
        pltpu.VMEM((NSEG, SEG, D), _F32),
        pltpu.SemaphoreType.DMA((NRB,)),
        pltpu.SemaphoreType.DMA((NFC,)),
        pltpu.SemaphoreType.DMA((NFC,)),
        pltpu.SemaphoreType.DMA((NT,)),
        pltpu.SemaphoreType.DMA((2, 3)),
        pltpu.SemaphoreType.DMA((NTF,)),
        pltpu.SemaphoreType.DMA((NT,)),
        pltpu.SemaphoreType.DMA((2,)),
    ]
    return kernel, scratch


@functools.partial(jax.jit, static_argnames=("A_seg_len",))
def pallas_parallel_sum__memory_aug_recurrent_mem_tr__dense_activation_gelu__prompt_kernel(
    A_x: jax.Array,
    A_mem0: jax.Array,
    A_Wq: jax.Array,
    A_Wk: jax.Array,
    A_Wv: jax.Array,
    A_Wo: jax.Array,
    A_seg_len: int,
    B_x: jax.Array,
    B_w1: jax.Array,
    B_b1: jax.Array,
    B_w2: jax.Array,
    B_b2: jax.Array,
):
    del B_x
    B, S, D = A_x.shape
    H, E = A_Wq.shape[1], A_Wq.shape[2]
    M = A_mem0.shape[1]
    SEG = int(A_seg_len)
    F = B_w1.shape[1]
    FT = 512
    FC = 384
    assert B == 1 and M == 8 and SEG == 32 and E == 128
    assert S % (8 * SEG) == 0 and D % 128 == 0 and H % 8 == 0
    assert (F - FT) % FC == 0 and (F - FT) // FC == D // 128
    NSEG = S // SEG

    scale = float(np.asarray(E ** (-0.5)).astype(A_x.dtype).astype(np.float32))

    kernel, scratch = _make_kernel(S, D, H, E, M, SEG, F, FC, FT, scale)

    vmem = pl.BlockSpec(memory_space=pltpu.VMEM)
    hbm = pl.BlockSpec(memory_space=pl.ANY)
    out = pl.pallas_call(
        kernel,
        out_shape=jax.ShapeDtypeStruct((NSEG, SEG, D), A_x.dtype),
        in_specs=[hbm, vmem, vmem, vmem, hbm, hbm, hbm, hbm, hbm, hbm],
        out_specs=hbm,
        scratch_shapes=scratch,
        compiler_params=pltpu.CompilerParams(vmem_limit_bytes=120 * 1024 * 1024),
    )(
        A_x.reshape(NSEG, SEG, D),
        A_mem0.reshape(M, D),
        B_b1.reshape(1, F),
        B_b2.reshape(1, D),
        A_Wq, A_Wk, A_Wv,
        A_Wo.reshape(H * E, D),
        B_w1, B_w2,
    )
    return out.reshape(B, S, D)
```

```python
import functools

import jax
import jax.numpy as jnp
import numpy as np
from jax import lax
from jax.experimental import pallas as pl
from jax.experimental.pallas import tpu as pltpu

_F32 = jnp.float32
_BF16 = jnp.bfloat16


def _dot(a, b):
    return jnp.dot(a, b, preferred_element_type=_F32)


def _dot_nt(a, b):
    return lax.dot_general(a, b, (((1,), (1,)), ((), ())), preferred_element_type=_F32)


def _make_kernel(S, D, H, E, M, SEG, F, FC, FT, scale):
    NSEG = S // SEG
    L = M + SEG
    LP = 48
    RIDE = 32 - M
    REST = SEG - RIDE
    NFC = (F - FT) // FC
    NTF = FT // 128
    F0 = NFC * FC
    NDC = D // 128
    NT = D // 128
    PH = 2
    NP = H // PH
    WLAG = 3
    SB = 8
    NRB = NSEG // SB
    RB = SB * SEG
    PB = 16
    NPB = NSEG // PB

    def kernel(x_hbm, mem0_ref, b1_ref, b2_ref,
               wq_hbm, wk_hbm, wv_hbm, wo_hbm, w1_hbm, w2_hbm,
               out_hbm,
               wqkv_v, wo_v, w1t_v, w2t_v, xn_v, xpre_v, acc_v,
               sem_x, sem_w1, sem_w2, sem_wo, sem_st, sem_w1t, sem_w2t, sem_out):
        w_hbm = (wq_hbm, wk_hbm, wv_hbm)

        def phase1(x_v, w1_v, w2_v, stage_v):
            def x_copy(i):
                r = pl.ds(i * SB, SB)
                return pltpu.make_async_copy(x_hbm.at[r], x_v.at[r], sem_x.at[i])

            def w1_copy(j):
                return pltpu.make_async_copy(
                    w1_hbm.at[:, pl.ds(j * FC, FC)], w1_v.at[j], sem_w1.at[j])

            def w2_copy(j):
                return pltpu.make_async_copy(
                    w2_hbm.at[pl.ds(j * FC, FC), :], w2_v.at[j], sem_w2.at[j])

            def st_copy(c, slot, p):
                return pltpu.make_async_copy(
                    w_hbm[p].at[pl.ds(c * 128, 128)], stage_v.at[slot, p],
                    sem_st.at[slot, p])

            def wo_copy(j):
                return pltpu.make_async_copy(
                    wo_hbm.at[:, pl.ds(j * 128, 128)], wo_v.at[j], sem_wo.at[j])

            def w1t_copy(t):
                return pltpu.make_async_copy(
                    w1_hbm.at[:, pl.ds(F0 + t * 128, 128)], w1t_v.at[t], sem_w1t.at[t])

            def w2t_copy(j):
                return pltpu.make_async_copy(
                    w2_hbm.at[pl.ds(F0, FT), pl.ds(j * 128, 128)], w2t_v.at[j],
                    sem_w2t.at[j])

            for i in range(NRB):
                x_copy(i).start()
            w1_copy(0).start()
            w2_copy(0).start()

            b2 = b2_ref[...].astype(_F32)

            def ln_body(i, carry):
                x_copy(i).wait()
                r = pl.ds(pl.multiple_of(i * SB, SB), SB)
                xb = x_v[r].astype(_F32)
                mu = jnp.mean(xb, axis=-1, keepdims=True)
                xc = xb - mu
                var = jnp.mean(xc * xc, axis=-1, keepdims=True)
                xn = xc * lax.rsqrt(var + 1e-5)
                xn_v[r] = xn.astype(_BF16)
                xpre_v[r] = xn[:, RIDE:, :]
                acc_v[r] = xb + b2
                return carry

            lax.fori_loop(0, NRB // 2, ln_body, 0)
            for p in range(3):
                st_copy(0, 0, p).start()
            w1_copy(1).start()
            w2_copy(1).start()
            for p in range(3):
                st_copy(1, 1, p).start()
            lax.fori_loop(NRB // 2, NRB, ln_body, 0)
            for j in range(2, NFC):
                w1_copy(j).start()
                w2_copy(j).start()
            for j in range(NT):
                wo_copy(j).start()
            for t in range(NTF):
                w1t_copy(t).start()
            for j in range(NT):
                w2t_copy(j).start()

            def relayout(c, slot, p, q):
                blk = stage_v[slot, p, pl.ds(q * 16, 16)]
                d0 = pl.multiple_of(c * 128 + q * 16, 16)
                wqkv_v[pl.ds(p * H, H), pl.ds(d0, 16), :] = jnp.swapaxes(blk, 0, 1)

            def fc_body(j, carry):
                slot = j % 2
                w1_copy(j).wait()
                w2_copy(j).wait()
                b1 = b1_ref[:, pl.ds(pl.multiple_of(j * FC, 128), FC)].astype(_F32)
                for rb in range(NRB):
                    if rb == 2:
                        for p in range(3):
                            st_copy(j, slot, p).wait()
                    xb = xn_v[pl.ds(rb * SB, SB)].reshape(RB, D)
                    u0 = 4 * (rb - 2)
                    if rb >= 2:
                        for u in range(u0, u0 + 2):
                            relayout(j, slot, u % 3, u // 3)
                    h = _dot(xb, w1_v[j]) + b1
                    h = jax.nn.gelu(h, approximate=True).astype(_BF16)
                    if rb >= 2:
                        for u in range(u0 + 2, u0 + 4):
                            relayout(j, slot, u % 3, u // 3)
                    y = _dot(h, w2_v[j])
                    acc_v[pl.ds(rb * SB, SB)] += y.reshape(SB, SEG, D)

                @pl.when(j + 2 < NDC)
                def _():
                    for p in range(3):
                        st_copy(j + 2, slot, p).start()

                return carry

            lax.fori_loop(0, NFC, fc_body, 0)
            for j in range(NT):
                wo_copy(j).wait()
                w2t_copy(j).wait()
            for t in range(NTF):
                w1t_copy(t).wait()

        pl.run_scoped(
            phase1,
            pltpu.VMEM((NSEG, SEG, D), _BF16),
            pltpu.VMEM((NFC, D, FC), _BF16),
            pltpu.VMEM((NFC, FC, D), _BF16),
            pltpu.VMEM((2, 3, 128, H, E), _BF16),
        )

        def phase2(qkvpre_v, opost_v, xl_v, wacc_v, obuf_v):
            xl_v[...] = xpre_v[...].reshape(NSEG * REST, D).astype(_BF16)

            def pre_body(sg, carry):
                for t in range(8):
                    slab = sg * 8 + t
                    y = _dot(xl_v[...], wqkv_v[slab])
                    qkvpre_v[slab] = y.reshape(NSEG, REST, E)
                return carry

            lax.fori_loop(0, 3 * H // 8, pre_body, 0)

            row = lax.broadcasted_iota(jnp.int32, (LP, LP), 0)
            col = lax.broadcasted_iota(jnp.int32, (LP, LP), 1)
            mask = ((row < M) | (row >= col)) & (col < L)
            zpad = jnp.zeros((LP - L, E), _F32)
            b1t = b1_ref[:, pl.ds(F0, FT)].astype(_F32)

            def seg_body(s, mem):
                xsb = xn_v[s]
                lhs = jnp.concatenate(
                    [mem, xsb.astype(_F32)[:RIDE]], axis=0).astype(_BF16)

                qkv = [{}, {}, {}]
                sc, mx, ex, den, pr, ob = {}, {}, {}, {}, {}, {}

                def heads(i):
                    return range(i * PH, (i + 1) * PH)

                def stage_a(p, i):
                    for h in heads(i):
                        y = _dot(lhs, wqkv_v[p * H + h])
                        qkv[p][h] = jnp.concatenate(
                            [y, qkvpre_v[p * H + h, s], zpad], axis=0).astype(_BF16)

                def stage_1(i):
                    for h in heads(i):
                        sc[h] = _dot_nt(qkv[0].pop(h), qkv[1].pop(h))

                def stage_2(i):
                    for h in heads(i):
                        sc[h] = jnp.where(mask, sc[h] * scale, -1000000000.0)
                        mx[h] = jnp.max(sc[h], axis=-1, keepdims=True)

                def stage_3(i):
                    for h in heads(i):
                        ex[h] = jnp.exp(sc.pop(h) - mx.pop(h))
                        den[h] = jnp.sum(ex[h], axis=-1, keepdims=True)

                def stage_4(i):
                    for h in heads(i):
                        d = den.pop(h)
                        r = pl.reciprocal(d, approx=True)
                        r = r * (2.0 - d * r)
                        pr[h] = (ex.pop(h) * r).astype(_BF16)

                def stage_5(i):
                    for h in heads(i):
                        o = _dot(pr.pop(h), qkv[2].pop(h))
                        ob[h] = o[:32].astype(_BF16)
                        opost_v[s, :, pl.ds(h * E, E)] = o[32:L]

                fin = []

                def stage_w(i):
                    og = jnp.concatenate([ob.pop(h) for h in heads(i)], axis=1)
                    for j in range(NT):
                        y = _dot(og, wo_v[j, pl.ds(i * PH * E, PH * E), :])
                        if i == 0:
                            wacc_v[:, pl.ds(j * 128, 128)] = y
                        elif i == NP - 1:
                            fin.append(wacc_v[:, pl.ds(j * 128, 128)] + y)
                        else:
                            wacc_v[:, pl.ds(j * 128, 128)] += y

                hm, ym, gl = {}, {}, []

                def stage_m1(t):
                    hm[t] = _dot(xsb, w1t_v[t])

                def stage_mg():
                    hh = jnp.concatenate([hm.pop(t) for t in range(NTF)], axis=1) + b1t
                    gl.append(jax.nn.gelu(hh, approximate=True).astype(_BF16))

                def stage_m2(j):
                    ym[j] = _dot(gl[0], w2t_v[j])

                for p in range(3):
                    stage_a(p, 0)
                for i in range(NP):
                    last = i == NP - 1
                    stage_1(i)
                    if last:
                        stage_w(i - 3)
                    else:
                        stage_a(0, i + 1)
                    stage_2(i)
                    if last:
                        stage_w(i - 2)
                    else:
                        stage_a(1, i + 1)
                    stage_3(i)
                    if last:
                        stage_w(i - 1)
                    else:
                        stage_a(2, i + 1)
                    stage_4(i)
                    if last:
                        for j in range(2, 5):
                            stage_m2(j)
                    elif i >= WLAG:
                        stage_w(i - WLAG)
                    elif i < 2:
                        stage_m1(2 * i)
                        stage_m1(2 * i + 1)
                    else:
                        stage_mg()
                        stage_m2(0)
                        stage_m2(1)
                    stage_5(i)
                for j in range(5, NT):
                    stage_m2(j)
                stage_w(NP - 1)

                out32 = jnp.concatenate(fin, axis=1)
                ymlp = jnp.concatenate([ym.pop(j) for j in range(NT)], axis=1)
                acc_v[s, pl.ds(0, RIDE), :] += out32[M:] + ymlp[:RIDE]
                acc_v[s, pl.ds(RIDE, REST), :] += ymlp[RIDE:]
                return out32[:M]

            lax.fori_loop(0, NSEG, seg_body, mem0_ref[...].astype(_F32))

            def out_copy(rb):
                return pltpu.make_async_copy(
                    obuf_v.at[rb % 2], out_hbm.at[pl.ds(rb * PB, PB)], sem_out.at[rb % 2])

            for rb in range(NPB):
                ol = opost_v[pl.ds(rb * PB, PB)].reshape(PB * REST, H * E).astype(_BF16)
                for j in range(NT):
                    y = _dot(ol, wo_v[j])
                    acc_v[pl.ds(rb * PB, PB), pl.ds(RIDE, REST), pl.ds(j * 128, 128)] += (
                        y.reshape(PB, REST, 128))
                if rb >= 2:
                    out_copy(rb - 2).wait()
                obuf_v[rb % 2] = acc_v[pl.ds(rb * PB, PB)].astype(obuf_v.dtype)
                out_copy(rb).start()
            for rb in range(NPB - 2, NPB):
                out_copy(rb).wait()

        pl.run_scoped(
            phase2,
            pltpu.VMEM((3 * H, NSEG, REST, E), _F32),
            pltpu.VMEM((NSEG, REST, H * E), _F32),
            pltpu.VMEM((NSEG * REST, D), _BF16),
            pltpu.VMEM((32, D), _F32),
            pltpu.VMEM((2, PB, SEG, D), _BF16),
        )

    scratch = [
        pltpu.VMEM((3 * H, D, E), _BF16),
        pltpu.VMEM((NT, H * E, 128), _BF16),
        pltpu.VMEM((NTF, D, 128), _BF16),
        pltpu.VMEM((NT, FT, 128), _BF16),
        pltpu.VMEM((NSEG, SEG, D), _BF16),
        pltpu.VMEM((NSEG, REST, D), _F32),
        pltpu.VMEM((NSEG, SEG, D), _F32),
        pltpu.SemaphoreType.DMA((NRB,)),
        pltpu.SemaphoreType.DMA((NFC,)),
        pltpu.SemaphoreType.DMA((NFC,)),
        pltpu.SemaphoreType.DMA((NT,)),
        pltpu.SemaphoreType.DMA((2, 3)),
        pltpu.SemaphoreType.DMA((NTF,)),
        pltpu.SemaphoreType.DMA((NT,)),
        pltpu.SemaphoreType.DMA((2,)),
    ]
    return kernel, scratch


@functools.partial(jax.jit, static_argnames=("A_seg_len",))
def pallas_parallel_sum__memory_aug_recurrent_mem_tr__dense_activation_gelu__prompt_kernel(
    A_x: jax.Array,
    A_mem0: jax.Array,
    A_Wq: jax.Array,
    A_Wk: jax.Array,
    A_Wv: jax.Array,
    A_Wo: jax.Array,
    A_seg_len: int,
    B_x: jax.Array,
    B_w1: jax.Array,
    B_b1: jax.Array,
    B_w2: jax.Array,
    B_b2: jax.Array,
):
    del B_x
    B, S, D = A_x.shape
    H, E = A_Wq.shape[1], A_Wq.shape[2]
    M = A_mem0.shape[1]
    SEG = int(A_seg_len)
    F = B_w1.shape[1]
    FT = 512
    FC = 384
    assert B == 1 and M == 8 and SEG == 32 and E == 128
    assert S % (8 * SEG) == 0 and D % 128 == 0 and H % 8 == 0
    assert (F - FT) % FC == 0 and (F - FT) // FC == D // 128
    NSEG = S // SEG

    scale = float(np.asarray(E ** (-0.5)).astype(A_x.dtype).astype(np.float32))

    kernel, scratch = _make_kernel(S, D, H, E, M, SEG, F, FC, FT, scale)

    vmem = pl.BlockSpec(memory_space=pltpu.VMEM)
    hbm = pl.BlockSpec(memory_space=pl.ANY)
    out = pl.pallas_call(
        kernel,
        out_shape=jax.ShapeDtypeStruct((NSEG, SEG, D), A_x.dtype),
        in_specs=[hbm, vmem, vmem, vmem, hbm, hbm, hbm, hbm, hbm, hbm],
        out_specs=hbm,
        scratch_shapes=scratch,
        compiler_params=pltpu.CompilerParams(vmem_limit_bytes=120 * 1024 * 1024),
    )(
        A_x.reshape(NSEG, SEG, D),
        A_mem0.reshape(M, D),
        B_b1.reshape(1, F),
        B_b2.reshape(1, D),
        A_Wq, A_Wk, A_Wv,
        A_Wo.reshape(H * E, D),
        B_w1, B_w2,
    )
    return out.reshape(B, S, D)
```

```python
import functools

import jax
import jax.numpy as jnp
import numpy as np
from jax import lax
from jax.experimental import pallas as pl
from jax.experimental.pallas import tpu as pltpu

_F32 = jnp.float32
_BF16 = jnp.bfloat16


def _dot(a, b):
    return jnp.dot(a, b, preferred_element_type=_F32)


def _dot_nt(a, b):
    return lax.dot_general(a, b, (((1,), (1,)), ((), ())), preferred_element_type=_F32)


def _make_kernel(S, D, H, E, M, SEG, F, FC, FT, scale):
    NSEG = S // SEG
    L = M + SEG
    RIDE = 32 - M
    REST = SEG - RIDE
    NFC = (F - FT) // FC
    NTF = FT // 128
    F0 = NFC * FC
    NDC = D // 128
    NT = D // 128
    PH = 2
    NP = H // PH
    WLAG = 3
    SB = 8
    NRB = NSEG // SB
    RB = SB * SEG
    PB = 16
    NPB = NSEG // PB

    def kernel(x_hbm, mem0_ref, b1_ref, b2_ref,
               wq_hbm, wk_hbm, wv_hbm, wo_hbm, w1_hbm, w2_hbm,
               out_hbm,
               wqkv_v, wo_v, w1t_v, w2t_v, xn_v, xpre_v, acc_v,
               sem_x, sem_w1, sem_w2, sem_wo, sem_st, sem_w1t, sem_w2t, sem_out):
        w_hbm = (wq_hbm, wk_hbm, wv_hbm)

        def phase1(x_v, w1_v, w2_v, stage_v):
            def x_copy(i):
                r = pl.ds(i * SB, SB)
                return pltpu.make_async_copy(x_hbm.at[r], x_v.at[r], sem_x.at[i])

            def w1_copy(j):
                return pltpu.make_async_copy(
                    w1_hbm.at[:, pl.ds(j * FC, FC)], w1_v.at[j], sem_w1.at[j])

            def w2_copy(j):
                return pltpu.make_async_copy(
                    w2_hbm.at[pl.ds(j * FC, FC), :], w2_v.at[j], sem_w2.at[j])

            def st_copy(c, slot, p):
                return pltpu.make_async_copy(
                    w_hbm[p].at[pl.ds(c * 128, 128)], stage_v.at[slot, p],
                    sem_st.at[slot, p])

            def wo_copy(j):
                return pltpu.make_async_copy(
                    wo_hbm.at[:, pl.ds(j * 128, 128)], wo_v.at[j], sem_wo.at[j])

            def w1t_copy(t):
                return pltpu.make_async_copy(
                    w1_hbm.at[:, pl.ds(F0 + t * 128, 128)], w1t_v.at[t], sem_w1t.at[t])

            def w2t_copy(j):
                return pltpu.make_async_copy(
                    w2_hbm.at[pl.ds(F0, FT), pl.ds(j * 128, 128)], w2t_v.at[j],
                    sem_w2t.at[j])

            for i in range(NRB):
                x_copy(i).start()
            w1_copy(0).start()
            w2_copy(0).start()

            b2 = b2_ref[...].astype(_F32)

            def ln_body(i, carry):
                x_copy(i).wait()
                r = pl.ds(pl.multiple_of(i * SB, SB), SB)
                xb = x_v[r].astype(_F32)
                mu = jnp.mean(xb, axis=-1, keepdims=True)
                xc = xb - mu
                var = jnp.mean(xc * xc, axis=-1, keepdims=True)
                xn = xc * lax.rsqrt(var + 1e-5)
                xn_v[r] = xn.astype(_BF16)
                xpre_v[r] = xn[:, RIDE:, :]
                acc_v[r] = xb + b2
                return carry

            lax.fori_loop(0, NRB // 2, ln_body, 0)
            for p in range(3):
                st_copy(0, 0, p).start()
            w1_copy(1).start()
            w2_copy(1).start()
            for p in range(3):
                st_copy(1, 1, p).start()
            lax.fori_loop(NRB // 2, NRB, ln_body, 0)
            for j in range(2, NFC):
                w1_copy(j).start()
                w2_copy(j).start()
            for j in range(NT):
                wo_copy(j).start()
            for t in range(NTF):
                w1t_copy(t).start()
            for j in range(NT):
                w2t_copy(j).start()

            def relayout(c, slot, p, q):
                blk = stage_v[slot, p, pl.ds(q * 16, 16)]
                d0 = pl.multiple_of(c * 128 + q * 16, 16)
                wqkv_v[pl.ds(p * H, H), pl.ds(d0, 16), :] = jnp.swapaxes(blk, 0, 1)

            def fc_body(j, carry):
                slot = j % 2
                w1_copy(j).wait()
                w2_copy(j).wait()
                b1 = b1_ref[:, pl.ds(pl.multiple_of(j * FC, 128), FC)].astype(_F32)
                for rb in range(NRB):
                    if rb == 2:
                        for p in range(3):
                            st_copy(j, slot, p).wait()
                    xb = xn_v[pl.ds(rb * SB, SB)].reshape(RB, D)
                    u0 = 4 * (rb - 2)
                    if rb >= 2:
                        for u in range(u0, u0 + 2):
                            relayout(j, slot, u % 3, u // 3)
                    h = _dot(xb, w1_v[j]) + b1
                    h = jax.nn.gelu(h, approximate=True).astype(_BF16)
                    if rb >= 2:
                        for u in range(u0 + 2, u0 + 4):
                            relayout(j, slot, u % 3, u // 3)
                    y = _dot(h, w2_v[j])
                    acc_v[pl.ds(rb * SB, SB)] += y.reshape(SB, SEG, D)

                @pl.when(j + 2 < NDC)
                def _():
                    for p in range(3):
                        st_copy(j + 2, slot, p).start()

                return carry

            lax.fori_loop(0, NFC, fc_body, 0)
            for j in range(NT):
                wo_copy(j).wait()
                w2t_copy(j).wait()
            for t in range(NTF):
                w1t_copy(t).wait()

        pl.run_scoped(
            phase1,
            pltpu.VMEM((NSEG, SEG, D), _BF16),
            pltpu.VMEM((NFC, D, FC), _BF16),
            pltpu.VMEM((NFC, FC, D), _BF16),
            pltpu.VMEM((2, 3, 128, H, E), _BF16),
        )

        def phase2(qkvpre_v, opost_v, xl_v, wacc_v, obuf_v):
            xl_v[...] = xpre_v[...].reshape(NSEG * REST, D).astype(_BF16)

            def pre_body(sg, carry):
                for t in range(8):
                    slab = sg * 8 + t
                    y = _dot(xl_v[...], wqkv_v[slab])
                    qkvpre_v[slab] = y.reshape(NSEG, REST, E)
                return carry

            lax.fori_loop(0, 3 * H // 8, pre_body, 0)

            row = lax.broadcasted_iota(jnp.int32, (PH * L, PH * L), 0)
            col = lax.broadcasted_iota(jnp.int32, (PH * L, PH * L), 1)
            row_hi, col_hi = row >= L, col >= L
            ri = jnp.where(row_hi, row - L, row)
            ci = jnp.where(col_hi, col - L, col)
            mask = (row_hi == col_hi) & ((ri < M) | (ri >= ci))
            b1t = b1_ref[:, pl.ds(F0, FT)].astype(_F32)

            def seg_body(s, mem):
                xsb = xn_v[s]
                lhs = jnp.concatenate(
                    [mem, xsb.astype(_F32)[:RIDE]], axis=0).astype(_BF16)

                qkv = [{}, {}, {}]
                sc, mx, ex, den, pr, ob = {}, {}, {}, {}, {}, {}

                def heads(i):
                    return range(i * PH, (i + 1) * PH)

                def stage_a(p, i):
                    parts = []
                    for h in heads(i):
                        parts.append(_dot(lhs, wqkv_v[p * H + h]))
                        parts.append(qkvpre_v[p * H + h, s])
                    qkv[p][i] = jnp.concatenate(parts, axis=0).astype(_BF16)

                def stage_1(i):
                    sc[i] = _dot_nt(qkv[0].pop(i), qkv[1].pop(i))

                def stage_2(i):
                    sc[i] = jnp.where(mask, sc[i] * scale, -1000000000.0)
                    mx[i] = jnp.max(sc[i], axis=-1, keepdims=True)

                def stage_3(i):
                    ex[i] = jnp.exp(sc.pop(i) - mx.pop(i))
                    den[i] = jnp.sum(ex[i], axis=-1, keepdims=True)

                def stage_4(i):
                    d = den.pop(i)
                    r = pl.reciprocal(d, approx=True)
                    r = r * (2.0 - d * r)
                    pr[i] = (ex.pop(i) * r).astype(_BF16)

                def stage_5(i):
                    o = _dot(pr.pop(i), qkv[2].pop(i))
                    ob[i] = jnp.concatenate(
                        [o[k * L:k * L + 32] for k in range(PH)], axis=1).astype(_BF16)
                    for k, h in enumerate(heads(i)):
                        opost_v[s, :, pl.ds(h * E, E)] = o[k * L + 32:(k + 1) * L]

                fin = []

                def stage_w(i):
                    og = ob.pop(i)
                    for j in range(NT):
                        y = _dot(og, wo_v[j, pl.ds(i * PH * E, PH * E), :])
                        if i == 0:
                            wacc_v[:, pl.ds(j * 128, 128)] = y
                        elif i == NP - 1:
                            fin.append(wacc_v[:, pl.ds(j * 128, 128)] + y)
                        else:
                            wacc_v[:, pl.ds(j * 128, 128)] += y

                hm, ym, gl = {}, {}, []

                def stage_m1(t):
                    hm[t] = _dot(xsb, w1t_v[t])

                def stage_mg():
                    hh = jnp.concatenate([hm.pop(t) for t in range(NTF)], axis=1) + b1t
                    gl.append(jax.nn.gelu(hh, approximate=True).astype(_BF16))

                def stage_m2(j):
                    ym[j] = _dot(gl[0], w2t_v[j])

                for p in range(3):
                    stage_a(p, 0)
                for i in range(NP):
                    last = i == NP - 1
                    stage_1(i)
                    if last:
                        stage_w(i - 3)
                    else:
                        stage_a(0, i + 1)
                    stage_2(i)
                    if last:
                        stage_w(i - 2)
                    else:
                        stage_a(1, i + 1)
                    stage_3(i)
                    if last:
                        stage_w(i - 1)
                    else:
                        stage_a(2, i + 1)
                    stage_4(i)
                    if last:
                        for j in range(2, 5):
                            stage_m2(j)
                    elif i >= WLAG:
                        stage_w(i - WLAG)
                    elif i < 2:
                        stage_m1(2 * i)
                        stage_m1(2 * i + 1)
                    else:
                        stage_mg()
                        stage_m2(0)
                        stage_m2(1)
                    stage_5(i)
                for j in range(5, NT):
                    stage_m2(j)
                stage_w(NP - 1)

                out32 = jnp.concatenate(fin, axis=1)
                ymlp = jnp.concatenate([ym.pop(j) for j in range(NT)], axis=1)
                acc_v[s, pl.ds(0, RIDE), :] += out32[M:] + ymlp[:RIDE]
                acc_v[s, pl.ds(RIDE, REST), :] += ymlp[RIDE:]
                return out32[:M]

            lax.fori_loop(0, NSEG, seg_body, mem0_ref[...].astype(_F32))

            def out_copy(rb):
                return pltpu.make_async_copy(
                    obuf_v.at[rb % 2], out_hbm.at[pl.ds(rb * PB, PB)], sem_out.at[rb % 2])

            for rb in range(NPB):
                ol = opost_v[pl.ds(rb * PB, PB)].reshape(PB * REST, H * E).astype(_BF16)
                for j in range(NT):
                    y = _dot(ol, wo_v[j])
                    acc_v[pl.ds(rb * PB, PB), pl.ds(RIDE, REST), pl.ds(j * 128, 128)] += (
                        y.reshape(PB, REST, 128))
                if rb >= 2:
                    out_copy(rb - 2).wait()
                obuf_v[rb % 2] = acc_v[pl.ds(rb * PB, PB)].astype(obuf_v.dtype)
                out_copy(rb).start()
            for rb in range(NPB - 2, NPB):
                out_copy(rb).wait()

        pl.run_scoped(
            phase2,
            pltpu.VMEM((3 * H, NSEG, REST, E), _F32),
            pltpu.VMEM((NSEG, REST, H * E), _F32),
            pltpu.VMEM((NSEG * REST, D), _BF16),
            pltpu.VMEM((32, D), _F32),
            pltpu.VMEM((2, PB, SEG, D), _BF16),
        )

    scratch = [
        pltpu.VMEM((3 * H, D, E), _BF16),
        pltpu.VMEM((NT, H * E, 128), _BF16),
        pltpu.VMEM((NTF, D, 128), _BF16),
        pltpu.VMEM((NT, FT, 128), _BF16),
        pltpu.VMEM((NSEG, SEG, D), _BF16),
        pltpu.VMEM((NSEG, REST, D), _F32),
        pltpu.VMEM((NSEG, SEG, D), _F32),
        pltpu.SemaphoreType.DMA((NRB,)),
        pltpu.SemaphoreType.DMA((NFC,)),
        pltpu.SemaphoreType.DMA((NFC,)),
        pltpu.SemaphoreType.DMA((NT,)),
        pltpu.SemaphoreType.DMA((2, 3)),
        pltpu.SemaphoreType.DMA((NTF,)),
        pltpu.SemaphoreType.DMA((NT,)),
        pltpu.SemaphoreType.DMA((2,)),
    ]
    return kernel, scratch


@functools.partial(jax.jit, static_argnames=("A_seg_len",))
def pallas_parallel_sum__memory_aug_recurrent_mem_tr__dense_activation_gelu__prompt_kernel(
    A_x: jax.Array,
    A_mem0: jax.Array,
    A_Wq: jax.Array,
    A_Wk: jax.Array,
    A_Wv: jax.Array,
    A_Wo: jax.Array,
    A_seg_len: int,
    B_x: jax.Array,
    B_w1: jax.Array,
    B_b1: jax.Array,
    B_w2: jax.Array,
    B_b2: jax.Array,
):
    del B_x
    B, S, D = A_x.shape
    H, E = A_Wq.shape[1], A_Wq.shape[2]
    M = A_mem0.shape[1]
    SEG = int(A_seg_len)
    F = B_w1.shape[1]
    FT = 512
    FC = 384
    assert B == 1 and M == 8 and SEG == 32 and E == 128
    assert S % (8 * SEG) == 0 and D % 128 == 0 and H % 8 == 0
    assert (F - FT) % FC == 0 and (F - FT) // FC == D // 128
    NSEG = S // SEG

    scale = float(np.asarray(E ** (-0.5)).astype(A_x.dtype).astype(np.float32))

    kernel, scratch = _make_kernel(S, D, H, E, M, SEG, F, FC, FT, scale)

    vmem = pl.BlockSpec(memory_space=pltpu.VMEM)
    hbm = pl.BlockSpec(memory_space=pl.ANY)
    out = pl.pallas_call(
        kernel,
        out_shape=jax.ShapeDtypeStruct((NSEG, SEG, D), A_x.dtype),
        in_specs=[hbm, vmem, vmem, vmem, hbm, hbm, hbm, hbm, hbm, hbm],
        out_specs=hbm,
        scratch_shapes=scratch,
        compiler_params=pltpu.CompilerParams(vmem_limit_bytes=120 * 1024 * 1024),
    )(
        A_x.reshape(NSEG, SEG, D),
        A_mem0.reshape(M, D),
        B_b1.reshape(1, F),
        B_b2.reshape(1, D),
        A_Wq, A_Wk, A_Wv,
        A_Wo.reshape(H * E, D),
        B_w1, B_w2,
    )
    return out.reshape(B, S, D)
```
